```python
import os as _os
_os.environ.setdefault("JAX_PLATFORMS", "cpu")
import jax
import jax.numpy as jnp

def _softmax(x, axis=-1):
    return jax.nn.softmax(x, axis=axis)
def _gelu(x):
    return jax.nn.gelu(x, approximate=True)
def _silu(x):
    return jax.nn.silu(x)
def _sigmoid(x):
    return jax.nn.sigmoid(x)
def _layernorm(x, axis=-1, eps=1e-5):
    m = jnp.mean(x, axis=axis, keepdims=True)
    v = jnp.var(x, axis=axis, keepdims=True)
    return (x - m) / jnp.sqrt(v + eps)
def _scatter_add(tgt, idx, src, axis=0):
    return tgt.at[idx].add(src)
def _segment_sum(src, seg, n):
    return jax.ops.segment_sum(src, seg, n)
class _Rng:
    def __init__(self, key):
        self._k = key
    def _next(self):
        self._k, sub = jax.random.split(self._k)
        return sub
    def normal(self, shape):
        return jax.random.normal(self._next(), shape, dtype=jnp.bfloat16)
    def randint(self, lo, hi, shape):
        return jax.random.randint(self._next(), shape, lo, hi, dtype=jnp.int32)
    def uniform(self, shape, lo=0.0, hi=1.0):
        return jax.random.uniform(self._next(), shape, jnp.bfloat16, lo, hi)
    def permutation(self, n):
        return jax.random.permutation(self._next(), n)


kernel_name = 'concat_heads__mha_block_cached__gqa_block_cached__near_ridge'

def setup_inputs():
    _rng = _Rng(jax.random.key(int.from_bytes(__import__("os").urandom(4), "little")))
    _w = (lambda a: (lambda t: t.astype(jnp.bfloat16) if jnp.issubdtype(t.dtype, jnp.floating) else t)(jnp.asarray(a)))
    def _A_setup():
        B, Sq, D = 16, 160, 512
        H, Sk, Dh = 32, 1024, 128
        return {
            "x": _w((lambda *s: _rng.normal(s) * 0.8)(B, Sq, D)),
            "k_cache": _w((lambda *s: _rng.normal(s) * 0.8)(B, H, Sk, Dh)),
            "v_cache": _w((lambda *s: _rng.normal(s) * 0.05)(B, H, Sk, Dh)),
            "wq": _w((lambda *s: _rng.normal(s) * 0.8)(D, H * Dh) * (D ** -0.5)),
            "wo": _w((lambda *s: _rng.normal(s) * 0.05)(H * Dh, D) * ((H * Dh) ** -0.5)),
        }
    _A_in = _A_setup()

    def _B_setup():
        B, Sq, D = 16, 160, 512
        Hq, Hkv, Sk, Dh = 32, 32, 1024, 128
        assert Hq % Hkv == 0, (Hq, Hkv)
        return {
            "x": _w((lambda *s: _rng.normal(s) * 0.8)(B, Sq, D)),
            "k_cache": _w((lambda *s: _rng.normal(s) * 0.8)(B, Hkv, Sk, Dh)),
            "v_cache": _w((lambda *s: _rng.normal(s) * 0.05)(B, Hkv, Sk, Dh)),
            "wq": _w((lambda *s: _rng.normal(s) * 0.8)(D, Hq * Dh) * (D ** -0.5)),
            "wo": _w((lambda *s: _rng.normal(s) * 0.05)(Hq * Dh, D) * ((Hq * Dh) ** -0.5)),
        }
    _B_in = _B_setup()

    return {
        "A_x": _A_in["x"],
        "A_k_cache": _A_in["k_cache"],
        "A_v_cache": _A_in["v_cache"],
        "A_wq": _A_in["wq"],
        "A_wo": _A_in["wo"],
        "B_x": _B_in["x"],
        "B_k_cache": _B_in["k_cache"],
        "B_v_cache": _B_in["v_cache"],
        "B_wq": _B_in["wq"],
        "B_wo": _B_in["wo"],
    }

def reference(A_x, A_k_cache, A_v_cache, A_wq, A_wo, B_x, B_k_cache, B_v_cache, B_wq, B_wo):
    def _A_ref(x, k_cache, v_cache, wq, wo):
        B, Sq, D = x.shape
        H, Dh = 32, 128
        q = (lambda x, *d: x.transpose(*d))((x @ wq).reshape(B, Sq, H, Dh), 0, 2, 1, 3)
        scores = jnp.einsum("bhqd,bhkd->bhqk", q, k_cache) * (Dh ** -0.5)
        p = _softmax(scores, axis=-1)
        o = jnp.einsum("bhqk,bhkd->bhqd", p, v_cache)
        return (lambda x, *d: x.transpose(*d))(o, 0, 2, 1, 3).reshape(B, Sq, H * Dh) @ wo

    def _B_ref(x, k_cache, v_cache, wq, wo):
        B, Sq, D = x.shape
        Hq, Dh = 32, 128
        Hkv = k_cache.shape[1]
        rep = Hq // Hkv
        q = (lambda x, *d: x.transpose(*d))((x @ wq).reshape(B, Sq, Hq, Dh), 0, 2, 1, 3)
        k = jnp.repeat(k_cache, rep, axis=1)
        v = jnp.repeat(v_cache, rep, axis=1)
        scores = jnp.einsum("bhqd,bhkd->bhqk", q, k) * (Dh ** -0.5)
        p = _softmax(scores, axis=-1)
        o = jnp.einsum("bhqk,bhkd->bhqd", p, v)
        return (lambda x, *d: x.transpose(*d))(o, 0, 2, 1, 3).reshape(B, Sq, Hq * Dh) @ wo

    a = _A_ref(A_x, A_k_cache, A_v_cache, A_wq, A_wo)
    b = _B_ref(B_x, B_k_cache, B_v_cache, B_wq, B_wo)
    return jnp.concatenate([a, b], axis=-1)
```

```python
import functools
import jax, jax.numpy as jnp
from jax import lax
import jax.experimental.pallas as pl
import jax.experimental.pallas.tpu as pltpu
B, Sq, D, H, Sk, Dh = 16, 160, 512, 32, 1024, 128
LOG2E = 1.4426950408889634
F32, BF16 = jnp.float32, jnp.bfloat16

def default_plan(GH, R=128):
    NP = Sk // R
    return [(2*k + hh, (i if hh == 0 else NP-1-i) * R) for k in range(GH//2) for i in range(NP) for hh in range(2)]

def make(GH=4, shift=16, opg=2, flags=None, nocompute=False, nodma=False, bitc=True, lags=(0,1,2,3), ostore=False,
         YR=16, yprio=True, plan=None, R=128, hord=None, wait_end=False, noout=False):
    NG = H // GH
    NIT = NG * B
    NB = 4
    plan = plan or default_plan(GH, R)
    WR = D // B
    OR = GH * Dh // B
    XR = 32
    G = 2 * GH
    hord = hord or [((t // 2) % 2, (t // 4) * 2 + t % 2) for t in range(G)]
    def kern(ax, ak, av, awq, awo, bx, bk, bv, bwq, bwo, o_hbm,
             xb, wqb, wob, kb, vb, ob, acc, obuf, kv_sem, w_sem, x_sem, o_sem):
        xs, ks, vs, wqs, wos = (ax, bx), (ak, bk), (av, bv), (awq, bwq), (awo, bwo)
        def ld(ref, idx):
            if bitc: return pltpu.bitcast(ref.bitcast(jnp.uint32)[idx], BF16)
            return ref[idx]
        def kv_piece(it, hh, r0):
            head = (it & (B - 1)) * H + (it >> 4) * GH + hh
            slot = it & (NB - 1)
            for br in range(2):
                pltpu.make_async_copy(ks[br].at[head, pl.ds(r0, R)], kb.at[slot, br, hh, pl.ds(r0, R)], kv_sem.at[slot]).start(priority=0)
                pltpu.make_async_copy(vs[br].at[head, pl.ds(r0, R)], vb.at[slot, br, hh, pl.ds(r0, R)], kv_sem.at[slot]).start(priority=1)
        def kv_wait(slot):
            pltpu.make_async_copy(kb.at[slot], kb.at[slot], kv_sem.at[slot]).wait()
            pltpu.make_async_copy(vb.at[slot], vb.at[slot], kv_sem.at[slot]).wait()
        def w_piece(g, i):
            ws = g & 1
            n = WR*4//GH
            for br in range(2):
                for r0 in range(0, WR, n):
                    rows = pl.ds(pl.multiple_of(i*WR + r0, n), n)
                    pltpu.make_async_copy(wqs[br].at[rows, pl.ds(pl.multiple_of(g*GH*Dh, GH*Dh), GH*Dh)], wqb.at[ws, br, rows], w_sem.at[0]).start(priority=0)
                for r0 in range(0, OR, min(OR, 32)):
                    m = min(OR, 32)
                    pltpu.make_async_copy(wos[br].at[pl.ds(pl.multiple_of(g*GH*Dh + i*OR + r0, m), m)], wob.at[ws, br, pl.ds(pl.multiple_of(i*OR + r0, m), m)], w_sem.at[0]).start(priority=1)
        def w_wait(ws):
            pltpu.make_async_copy(wqb.at[ws], wqb.at[ws], w_sem.at[0]).wait()
            pltpu.make_async_copy(wob.at[ws], wob.at[ws], w_sem.at[0]).wait()
        def x_start(b):
            for r0 in range(0, Sq, XR):
                for br in range(2):
                    pltpu.make_async_copy(xs[br].at[b, pl.ds(r0, XR)], xb.at[b, br, pl.ds(r0, XR)], x_sem.at[0]).start(priority=br)
        def x_wait(b):
            pltpu.make_async_copy(xb.at[b], xb.at[b], x_sem.at[0]).wait()
        def o_rows(b0, nb):
            if YR > Sq:
                pltpu.make_async_copy(ob.at[pl.ds(b0, nb)], o_hbm.at[pl.ds(b0, nb)], o_sem.at[0]).start()
                return
            n = 0
            for i in range(Sq // YR):
                for b in range(b0, b0 + nb):
                    pltpu.make_async_copy(ob.at[b, pl.ds(i*YR, YR)], o_hbm.at[b, pl.ds(i*YR, YR)], o_sem.at[0]).start(priority=n % 2 if yprio else 0)
                    n += 1

        x_start(0)
        lax.fori_loop(0, B, lambda i, _: w_piece(0, i), None)
        for hh, r0 in plan: kv_piece(0, hh, r0)
        if not nodma:
            for hh, r0 in plan[:shift]: kv_piece(1, hh, r0)
        def waits(it):
            g, b = it >> 4, it & (B - 1)
            pl.when(g == 0)(lambda: x_wait(b))
            pl.when(b == 0)(lambda: w_wait(g & 1))
            kv_wait(it & (NB - 1))
        if nodma or wait_end:
            x_wait(0); w_wait(0); kv_wait(0)

        def step(it, _):
            g, b = it >> 4, it & (B - 1)
            ws = g & 1
            s0 = it & (NB - 1)
            todo = []
            if not nodma:
                if not wait_end: waits(it)
                todo.append(lambda: pl.when(it < B - 1)(lambda: x_start(b + 1)))
                todo.append(lambda: pl.when(g < NG - 1)(lambda: w_piece(g + 1, b)))
                for d, part in ((1, plan[shift:]), (2, plan[:shift])):
                    for hh, r0 in part:
                        todo.append(functools.partial(lambda d, hh, r0: pl.when(it < NIT - d)(lambda: kv_piece(it + d, hh, r0)), d, hh, r0))
                    if d == 1 and not noout:
                        for b0 in range(0, B-2, 2):
                            todo.append(functools.partial(lambda b0: pl.when(it == NIT - 2 + (b0 >= 6))(lambda: o_rows(b0, 2)), b0))
            ntodo = len(todo)
            done = [0]
            def issue(frac):
                want = ntodo * done[0] // (6*G - 8)
                done[0] += frac
                while todo and ntodo - len(todo) < want: todo.pop(0)()
            if nocompute:
                issue(6*G); issue(0)
            else:
                def qp(t):
                    br, h = hord[t]
                    q = jnp.dot(xb[b, br], wqb[ws, br, :, h*Dh:(h+1)*Dh], preferred_element_type=F32)
                    return (q * (Dh**-0.5 * LOG2E)).astype(BF16)
                def qk(t, q):
                    return lax.dot_general(q, ld(kb, (s0, *hord[t])), (((1,),(1,)),((),())), preferred_element_type=F32)
                def sm(s):
                    m = jnp.max(s, axis=-1, keepdims=True)
                    p = jnp.exp2(s - m)
                    return p.astype(BF16), jnp.sum(p, axis=-1, keepdims=True)
                def pv(t, p, l):
                    br, h = hord[t]
                    o = jnp.dot(p, ld(vb, (s0, br, h)), preferred_element_type=F32)
                    o = (o * pltpu.reciprocal(l, full_range=False)).astype(BF16)
                    if ostore:
                        obuf[br, :, h*Dh:(h+1)*Dh] = o
                        return None
                    return o
                q, p, o = {}, {}, {}
                tot = [None, None]
                for t in range(G + max(lags)):
                    if 0 <= t - lags[0] < G: issue(1); q[t-lags[0]] = qp(t-lags[0])
                    if 0 <= t - lags[1] < G: issue(2); p[t-lags[1]] = sm(qk(t-lags[1], q.pop(t-lags[1])))
                    if 0 <= t - lags[2] < G:
                        tt = t - lags[2]
                        issue(2); o[hord[tt]] = pv(tt, *p.pop(tt))
                    tt = t - lags[3]
                    if 0 <= tt < G and (hord[tt][1] + 1) % opg == 0:
                        issue(opg)
                        br, h1 = hord[tt][0], hord[tt][1] + 1
                        os = [o.pop((br, i)) for i in range(h1 - opg, h1)]
                        if ostore: oo = obuf[br, :, (h1-opg)*Dh:h1*Dh]
                        else: oo = os[0] if opg == 1 else jnp.concatenate(os, axis=1)
                        r = jnp.dot(oo, wob[ws, br, (h1-opg)*Dh:h1*Dh, :], preferred_element_type=F32)
                        if tot[br] is None: tot[br] = jnp.where(g == 0, 0.0, acc[b, br])
                        tot[br] = tot[br] + r
                        if h1 == GH:
                            acc[b, br] = tot[br]
                            ob[b, :, br*D:(br+1)*D] = tot[br].astype(BF16)
            assert not todo
            if wait_end and not nodma: pl.when(it < NIT - 1)(lambda: waits(it + 1))

        lax.fori_loop(0, NIT, step, None)
        if nodma or noout:
            o_rows(0, 1)
            pltpu.make_async_copy(ob.at[0], o_hbm.at[0], o_sem.at[0]).wait()
        else:
            o_rows(B - 2, 2)
            pltpu.make_async_copy(ob, o_hbm, o_sem.at[0]).wait()

    def fn(ax, ak, av, awq, awo, bx, bk, bv, bwq, bwo):
        r = lambda t: t.reshape(B*H, Sk, Dh)
        return pl.pallas_call(kern,
            in_specs=[pl.BlockSpec(memory_space=pl.ANY)]*10,
            out_specs=pl.BlockSpec(memory_space=pl.ANY),
            out_shape=jax.ShapeDtypeStruct((B,Sq,2*D), BF16),
            scratch_shapes=[pltpu.VMEM((B,2,Sq,D), BF16), pltpu.VMEM((2,2,D,GH*Dh), BF16), pltpu.VMEM((2,2,GH*Dh,D), BF16),
                            pltpu.VMEM((NB,2,GH,Sk,Dh), BF16), pltpu.VMEM((NB,2,GH,Sk,Dh), BF16),
                            pltpu.VMEM((B,Sq,2*D), BF16), pltpu.VMEM((B,2,Sq,D), F32), pltpu.VMEM((2,Sq,GH*Dh), BF16),
                            pltpu.SemaphoreType.DMA((NB,)), pltpu.SemaphoreType.DMA((1,)), pltpu.SemaphoreType.DMA((1,)), pltpu.SemaphoreType.DMA((1,))],
            compiler_params=pltpu.CompilerParams(vmem_limit_bytes=110*2**20, flags=flags, disable_bounds_checks=True),
        )(ax, r(ak), r(av), awq, awo, bx, r(bk), r(bv), bwq, bwo)
    return fn


_impl = make(YR=160)

@jax.jit
def pallas_concat_heads__mha_block_cached__gqa_block_cached__near_ridge_kernel(
    A_x, A_k_cache, A_v_cache, A_wq, A_wo, B_x, B_k_cache, B_v_cache, B_wq, B_wo):
    return _impl(A_x, A_k_cache, A_v_cache, A_wq, A_wo, B_x, B_k_cache, B_v_cache, B_wq, B_wo)
```

```python
import functools

import jax
import jax.numpy as jnp
from jax import lax
import jax.experimental.pallas as pl
import jax.experimental.pallas.tpu as pltpu

F32, BF16 = jnp.float32, jnp.bfloat16
LOG2E = 1.4426950408889634
LANES = 128

QUAD = 4
SLOTS = 4
WQ_HEADS = 4
KV_ROWS = 128
ROWS = 32

AHEAD = (8, 40)
EARLY_OUT = 16

SCHEDULE = ("q0 q1 q2 k0 k1 v0 q3 o0 k2 v1 q4 k3 k4 v2 q5 o1 "
            "q6 o2 v3 q7 o3 k5 v4 k6 k7 v5 o4 v6 o5 v7 o6 o7").split()
MXU_COST = {"q": 1, "k": 2, "v": 2, "o": 1}
PREFETCH_SPAN = 39


def _batch(quad, i):
    return (quad >> 1) * 8 + (quad & 1) + 2 * i


def _start_all(copies):
    for n, copy in enumerate(copies):
        copy.start(priority=n % 2)


def _wait_filled(buf, sem):
    pltpu.make_async_copy(buf, buf, sem).wait()


def _kernel(ax, ak, av, awq, awo, bx, bk, bv, bwq, bwo, out_hbm,
            x_buf, wq_buf, wo_buf, kv_buf, p_buf, l_buf, acc, out_buf,
            kv_sem, x_sem, wq_sem, wo_sem, out_sem):
    n_batch, sq, d = ax.shape
    _, _, sk, dh = ak.shape
    heads = awq.shape[1] // dh
    n_steps = heads * QUAD
    wq_steps = WQ_HEADS * QUAD
    assert n_batch == QUAD * QUAD == wq_steps and heads % WQ_HEADS == 0
    assert d == wq_steps * ROWS and dh == QUAD * ROWS
    assert sq % ROWS == 0 and sk % KV_ROWS == 0
    x_hbm, wq_hbm, wo_hbm = (ax, bx), (awq, bwq), (awo, bwo)
    kv_hbm = ((ak, bk), (av, bv))

    def start_kv(kv, step, br, i, row, priority):
        src = kv_hbm[kv][br]
        head = step >> 2
        if src.shape[1] != heads:
            head = head // (heads // src.shape[1])
        slot = step & (SLOTS - 1)
        rows = pl.ds(row, KV_ROWS)
        pltpu.make_async_copy(
            src.at[_batch(step & (QUAD - 1), i), head, rows],
            kv_buf.at[slot, kv, br, i, rows], kv_sem.at[slot]).start(priority=priority)

    def start_x(quad, i, row):
        rows = pl.ds(row, ROWS)
        _start_all([pltpu.make_async_copy(
            x_hbm[br].at[_batch(quad, i), rows], x_buf.at[quad, br, i, rows], x_sem)
            for br in range(2)])

    def start_wq(group, part):
        rows = pl.ds(pl.multiple_of(part * ROWS, ROWS), ROWS)
        cols = pl.ds(pl.multiple_of(group * WQ_HEADS * dh, dh), WQ_HEADS * dh)
        _start_all([pltpu.make_async_copy(
            wq_hbm[br].at[rows, cols], wq_buf.at[group & 1, br, rows], wq_sem)
            for br in range(2)])

    def start_wo(head, part):
        src = pl.ds(pl.multiple_of(head * dh + part * ROWS, ROWS), ROWS)
        dst = pl.ds(pl.multiple_of(part * ROWS, ROWS), ROWS)
        _start_all([pltpu.make_async_copy(
            wo_hbm[br].at[src], wo_buf.at[head & 1, br, dst], wo_sem)
            for br in range(2)])

    def start_out(pieces):
        _start_all([pltpu.make_async_copy(
            out_buf.at[b, pl.ds(r, ROWS)], out_hbm.at[b, pl.ds(r, ROWS)], out_sem)
            for b, r in pieces])

    def out_pieces(quads, members=range(QUAD)):
        return [(_batch(quad, i), r)
                for r in range(0, sq, ROWS) for quad in quads for i in members]

    kv_pieces = [(br, i, r) for r in range(0, sk, KV_ROWS)
                 for br in range(2) for i in range(QUAD)]
    x_pieces = [(i, r) for r in range(0, sq, ROWS) for i in range(QUAD)]

    out_early = out_pieces((0, 1))[:EARLY_OUT]
    out_last = [piece for _, piece in sorted(
        ((n + 0.5) / len(part), piece)
        for part in (out_pieces((0, 1))[EARLY_OUT:], out_pieces((2,)))
        for n, piece in enumerate(part))]

    for piece in x_pieces:
        start_x(0, *piece)

    def first_wq(part, _):
        start_wq(0, part)
        acc[part] = jnp.zeros(acc.shape[1:], F32)
    lax.fori_loop(0, wq_steps, first_wq, None)

    for part in range(QUAD):
        start_wo(0, part)

    def first_kv(n, _):
        row = pl.multiple_of(n * KV_ROWS, KV_ROWS)
        for br in range(2):
            for i in range(QUAD):
                for kv in range(2):
                    start_kv(kv, 0, br, i, row, kv)
    lax.fori_loop(0, sk // KV_ROWS, first_kv, None)

    head_start = [(kv, piece) for n, piece in enumerate(kv_pieces)
                  for kv in range(2) if n < AHEAD[kv]]
    for n, (kv, piece) in enumerate(head_start):
        start_kv(kv, 1, *piece, n % 2)

    def step(it, _):
        head, quad = it >> 2, it & (QUAD - 1)
        group, part = it >> 4, it & (wq_steps - 1)
        slot = it & (SLOTS - 1)
        last = it == n_steps - 1

        pl.when(head == 0)(lambda: _wait_filled(x_buf.at[quad], x_sem))
        pl.when(part == 0)(lambda: _wait_filled(wq_buf.at[group & 1], wq_sem))
        pl.when(quad == 0)(lambda: _wait_filled(wo_buf.at[head & 1], wo_sem))
        _wait_filled(kv_buf.at[slot], kv_sem.at[slot])
        pl.when(last)(lambda: start_out(out_last))

        def prefetch(n):
            for kv in range(2):
                later, m = divmod(n + AHEAD[kv], len(kv_pieces))
                pl.when(it < n_steps - 1 - later)(functools.partial(
                    start_kv, kv, it + 1 + later, *kv_pieces[m], kv))
            if n < len(x_pieces):
                pl.when(it < QUAD - 1)(lambda: start_x(quad + 1, *x_pieces[n]))
            if n == 0:
                pl.when(it < n_steps - wq_steps)(lambda: start_wq(group + 1, part))
                pl.when(it < n_steps - QUAD)(lambda: start_wo(head + 1, quad))
            first = EARLY_OUT - 4 * (len(kv_pieces) - n)
            if first >= 0:
                pl.when(it == n_steps - 2)(
                    lambda: start_out(out_early[first:first + 4]))

        wq_cols = pl.ds(pl.multiple_of((head & (WQ_HEADS - 1)) * dh, dh), dh)
        started = cost = 0
        live = {}
        for kind, t in SCHEDULE:
            due = len(kv_pieces) * min(cost, PREFETCH_SPAN) // PREFETCH_SPAN
            for n in range(started, due):
                prefetch(n)
            started = due
            cost += MXU_COST[kind]

            t = int(t)
            i, br = divmod(t, 2)
            if kind == "q":
                q = jnp.dot(x_buf[quad, br, i], wq_buf[group & 1, br, :, wq_cols],
                            preferred_element_type=F32)
                live[t] = (q * (dh ** -0.5 * LOG2E)).astype(BF16)
            elif kind == "k":
                s = lax.dot_general(live.pop(t), kv_buf[slot, 0, br, i],
                                    (((1,), (1,)), ((), ())),
                                    preferred_element_type=F32)
                p = jnp.exp2(s - jnp.max(s, axis=-1, keepdims=True))
                l_buf[t] = functools.reduce(
                    jnp.add, [p[:, c:c + LANES] for c in range(0, sk, LANES)])
                p_buf[t] = p.astype(BF16)
            elif kind == "v":
                o = jnp.dot(p_buf[t], kv_buf[slot, 1, br, i],
                            preferred_element_type=F32)
                l = jnp.sum(l_buf[t], axis=-1, keepdims=True)
                live[t] = (o * (1.0 / l)).astype(BF16)
            else:
                b = _batch(quad, i)
                total = acc[b, br] + jnp.dot(live.pop(t), wo_buf[head & 1, br],
                                             preferred_element_type=F32)
                acc[b, br] = total
                out_buf[b, :, br * d:(br + 1) * d] = total.astype(out_buf.dtype)
                if br == 1 and i < QUAD - 1:
                    pl.when(last)(functools.partial(
                        start_out, out_pieces((QUAD - 1,), (i,))))
        assert started == len(kv_pieces)

    lax.fori_loop(0, n_steps, step, None)

    start_out(out_pieces((QUAD - 1,), (QUAD - 1,)))
    pltpu.make_async_copy(out_buf, out_hbm, out_sem).wait()


@jax.jit
def pallas_concat_heads__mha_block_cached__gqa_block_cached__near_ridge_kernel(
    A_x: jax.Array,
    A_k_cache: jax.Array,
    A_v_cache: jax.Array,
    A_wq: jax.Array,
    A_wo: jax.Array,
    B_x: jax.Array,
    B_k_cache: jax.Array,
    B_v_cache: jax.Array,
    B_wq: jax.Array,
    B_wo: jax.Array,
):
    n_batch, sq, d = A_x.shape
    _, _, sk, dh = A_k_cache.shape
    dtype = A_x.dtype
    return pl.pallas_call(
        _kernel,
        in_specs=[pl.BlockSpec(memory_space=pl.ANY)] * 10,
        out_specs=pl.BlockSpec(memory_space=pl.ANY),
        out_shape=jax.ShapeDtypeStruct((n_batch, sq, 2 * d), dtype),
        scratch_shapes=[
            pltpu.VMEM((QUAD, 2, QUAD, sq, d), dtype),
            pltpu.VMEM((2, 2, d, WQ_HEADS * dh), dtype),
            pltpu.VMEM((2, 2, dh, d), dtype),
            pltpu.VMEM((SLOTS, 2, 2, QUAD, sk, dh), dtype),
            pltpu.VMEM((2 * QUAD, sq, sk), BF16),
            pltpu.VMEM((2 * QUAD, sq, LANES), F32),
            pltpu.VMEM((n_batch, 2, sq, d), F32),
            pltpu.VMEM((n_batch, sq, 2 * d), dtype),
            pltpu.SemaphoreType.DMA((SLOTS,)),
            pltpu.SemaphoreType.DMA(()),
            pltpu.SemaphoreType.DMA(()),
            pltpu.SemaphoreType.DMA(()),
            pltpu.SemaphoreType.DMA(()),
        ],
        compiler_params=pltpu.CompilerParams(
            vmem_limit_bytes=64 * 2**20,
            disable_bounds_checks=True,
        ),
    )(A_x, A_k_cache, A_v_cache, A_wq, A_wo, B_x, B_k_cache, B_v_cache, B_wq, B_wo)
```
